```python
import jax
import jax.numpy as jnp

def _softmax(x, axis=-1):
    return jax.nn.softmax(x, axis=axis)

def _gelu(x):
    return jax.nn.gelu(x, approximate=True)

def _silu(x):
    return jax.nn.silu(x)

def _sigmoid(x):
    return jax.nn.sigmoid(x)

def _layernorm(x, axis=-1, eps=1e-05):
    m = jnp.mean(x, axis=axis, keepdims=True)
    v = jnp.var(x, axis=axis, keepdims=True)
    return (x - m) / jnp.sqrt(v + eps)

def _scatter_add(tgt, idx, src, axis=0):
    return tgt.at[idx].add(src)

def _segment_sum(src, seg, n):
    return jax.ops.segment_sum(src, seg, n)

class _Rng:

    def __init__(self, key):
        self._k = key

    def _next(self):
        self._k, sub = jax.random.split(self._k)
        return sub

    def normal(self, shape):
        return jax.random.normal(self._next(), shape, dtype=jnp.bfloat16)

    def randint(self, lo, hi, shape):
        return jax.random.randint(self._next(), shape, lo, hi, dtype=jnp.int32)

    def uniform(self, shape, lo=0.0, hi=1.0):
        return jax.random.uniform(self._next(), shape, jnp.bfloat16, lo, hi)

    def permutation(self, n):
        return jax.random.permutation(self._next(), n)
kernel_name = 'interleave_layers__linear_kernel_hedgehog__memory_aug_recurrent_mem_tr__prompt'

def setup_inputs():
    _rng = _Rng(jax.random.key(int.from_bytes(__import__("os").urandom(4), "little")))
    _w = lambda a: (lambda t: t.astype(jnp.bfloat16) if jnp.issubdtype(t.dtype, jnp.floating) else t)(jnp.asarray(a))

    def _A_setup():
        B, S, D, H = (1, 2048, 640, 32)
        Dh = D // H
        return {'x': _w((lambda *s: _rng.normal(s) * 0.05)(B, S, D)), 'wqkv': _w((lambda *s: _rng.normal(s) * 0.05)(D, 3 * D)), 'w_phi': _w((lambda *s: _rng.normal(s) * 0.05)(H, Dh, Dh) * Dh ** (-0.5)), 'wo': _w((lambda *s: _rng.normal(s) * 0.05)(D, D))}
    _A_in = _A_setup()

    def _B_setup():
        B, S, Dm = (1, 2048, 640)
        H, Dh = (32, 192)
        M, seg = (8, 32)
        seg = min(seg, S)
        S = S // seg * seg
        return {'x': _w((lambda *s: _rng.normal(s) * 0.05)(B, S, Dm)), 'mem0': _w((lambda *s: _rng.normal(s) * 0.05)(B, M, Dm)), 'Wq': _w((lambda *s: _rng.normal(s) * 0.05)(Dm, H, Dh) * Dm ** (-0.5)), 'Wk': _w((lambda *s: _rng.normal(s) * 0.05)(Dm, H, Dh) * Dm ** (-0.5)), 'Wv': _w((lambda *s: _rng.normal(s) * 0.05)(Dm, H, Dh) * Dm ** (-0.5)), 'Wo': _w((lambda *s: _rng.normal(s) * 0.05)(H, Dh, Dm) * (H * Dh) ** (-0.5)), 'seg_len': seg}
    _B_in = _B_setup()
    return {'A_x': _A_in['x'], 'A_wqkv': _A_in['wqkv'], 'A_w_phi': _A_in['w_phi'], 'A_wo': _A_in['wo'], 'B_x': _B_in['x'], 'B_mem0': _B_in['mem0'], 'B_Wq': _B_in['Wq'], 'B_Wk': _B_in['Wk'], 'B_Wv': _B_in['Wv'], 'B_Wo': _B_in['Wo'], 'B_seg_len': _B_in['seg_len']}

def reference(A_x, A_wqkv, A_w_phi, A_wo, B_x, B_mem0, B_Wq, B_Wk, B_Wv, B_Wo, B_seg_len):

    def _A_ref(x, wqkv, w_phi, wo):
        B, S, D = x.shape
        H = 32
        Dh = D // H
        qkv = (lambda x, *d: x.transpose(*d))((x @ wqkv).reshape(B, S, 3, H, Dh), 2, 0, 3, 1, 4)
        q, k, v = (qkv[0], qkv[1], qkv[2])
        pq = jnp.einsum('bhsd,hdf->bhsf', q, w_phi)
        pk = jnp.einsum('bhsd,hdf->bhsf', k, w_phi)
        phi_q = jnp.concatenate([_softmax(pq, axis=-1), _softmax(-pq, axis=-1)], axis=-1)
        phi_k = jnp.concatenate([_softmax(pk, axis=-1), _softmax(-pk, axis=-1)], axis=-1)
        kv = jnp.einsum('bhsf,bhsd->bhfd', phi_k, v)
        z = jnp.einsum('bhsf->bhf', phi_k)
        num = jnp.einsum('bhqf,bhfd->bhqd', phi_q, kv)
        den = jnp.einsum('bhqf,bhf->bhq', phi_q, z)[..., None] + 1e-06
        o = num / den
        return (lambda x, *d: x.transpose(*d))(o, 0, 2, 1, 3).reshape(B, S, D) @ wo

    def _B_ref(x, mem0, Wq, Wk, Wv, Wo, seg_len):
        B, S, Dm = x.shape
        H, Dh = (Wq.shape[1], Wq.shape[2])
        M = mem0.shape[1]
        scale = Dh ** (-0.5)
        n_seg = S // seg_len
        L = M + seg_len
        idx = jnp.arange(L)
        mask = (idx[:, None] < M) | (idx[:, None] >= idx[None, :])
        mem = mem0
        outs = []
        for s in range(n_seg):
            xs = x[:, s * seg_len:(s + 1) * seg_len, :].copy()
            h = jnp.concatenate([mem, xs], axis=1)
            q = jnp.einsum('btd,dhe->bhte', h, Wq)
            k = jnp.einsum('btd,dhe->bhte', h, Wk)
            v = jnp.einsum('btd,dhe->bhte', h, Wv)
            scores = jnp.einsum('bhqe,bhke->bhqk', q, k) * scale
            scores = jnp.where(mask[None, None], scores, -1000000000.0)
            p = _softmax(scores, axis=-1)
            o = jnp.einsum('bhqk,bhke->bhqe', p, v)
            o = jnp.einsum('bhte,hed->btd', o, Wo)
            mem = o[:, :M, :].copy()
            outs.append(o[:, M:, :])
        return jnp.concatenate(outs, axis=1)
    x = A_x
    x = x + _A_ref(_layernorm(x, axis=-1), A_wqkv, A_w_phi, A_wo)
    x = x + _B_ref(_layernorm(x, axis=-1), B_mem0, B_Wq, B_Wk, B_Wv, B_Wo, B_seg_len)
    x = x + _A_ref(_layernorm(x, axis=-1), A_wqkv, A_w_phi, A_wo)
    x = x + _B_ref(_layernorm(x, axis=-1), B_mem0, B_Wq, B_Wk, B_Wv, B_Wo, B_seg_len)
    return x
```

```python
import jax
import jax.numpy as jnp
from jax import lax
import jax.experimental.pallas as pl
import jax.experimental.pallas.tpu as pltpu

F32 = jnp.float32
BF16 = jnp.bfloat16

S, D = 2048, 640
AH, AD = 32, 20
BH, BD = 32, 192
M, SEG = 8, 32
L = M + SEG
HD = BH * BD
NP = BH // 2
PW = 2 * BD
RB = 256
NT = D // 128


def _dot(a, b):
    return lax.dot_general(a, b, (((1,), (0,)), ((), ())), preferred_element_type=F32)


def _dot_nt(a, b):
    return lax.dot_general(a, b, (((1,), (1,)), ((), ())), preferred_element_type=F32)


def _dot_tn(a, b):
    return lax.dot_general(a, b, (((0,), (0,)), ((), ())), preferred_element_type=F32)


def _ln(x):
    m = jnp.mean(x, axis=-1, keepdims=True)
    c = x - m
    v = jnp.mean(c * c, axis=-1, keepdims=True)
    return c * lax.rsqrt(v + 1e-5)


def _tiles(x):
    return [x[:, t * 128:(t + 1) * 128] for t in range(x.shape[1] // 128)]


def _group(op, tiles):
    t = tiles[0]
    for u in tiles[1:]:
        t = op(t, u)
    t = op(t, pltpu.roll(t, 64, 1))
    return op(t, pltpu.roll(t, 32, 1))


def _phi(p):
    ts = _tiles(p)
    mx = _group(jnp.maximum, ts)
    mn = _group(jnp.minimum, ts)
    ep = [jnp.exp(t - mx) for t in ts]
    en = [jnp.exp(mn - t) for t in ts]
    rp = 1.0 / _group(jnp.add, ep)
    rn = 1.0 / _group(jnp.add, en)
    return [e * rp for e in ep] + [e * rn for e in en]


def _kernel(x_ref, wqkv_ref, wp_ref, awo_ref, mem0_ref, wq_h, wk_h, wv_h, wo_h,
            o_ref,
            xs, xn, aw, awo, phq, kvt, kvm, wpp, stage, bw, bwo, osc, sems):
    cps = [pltpu.make_async_copy(src, stage.at[i], sems.at[i])
           for i, src in enumerate((wq_h, wk_h, wv_h))]
    cps.append(pltpu.make_async_copy(wo_h, bwo, sems.at[3]))
    for c in cps:
        c.start()

    r = lax.broadcasted_iota(jnp.int32, (D, D), 0)
    c = lax.broadcasted_iota(jnp.int32, (D, D), 1)
    rh = (r * 3277) >> 16
    rd = r - rh * AD
    same = (c & 31) == rh
    wpp[...] = jnp.zeros(wpp.shape, BF16)
    wpp[0:AD, :] = wp_ref[...]
    r1 = lax.broadcasted_iota(jnp.int32, (D, 128), 0)
    c1 = lax.broadcasted_iota(jnp.int32, (D, 128), 1)
    sel = jnp.where(r1 - ((r1 * 3277) >> 16) * AD == c1, 1.0, 0.0).astype(BF16)
    bd = jnp.where(same, _dot(sel, wpp[...]), 0.0).astype(BF16)
    perm = jnp.where(same & ((c >> 5) == rd), 1.0, 0.0).astype(BF16)
    aw[:, 0:D] = _dot(wqkv_ref[:, 0:D], bd).astype(BF16)
    aw[:, D:2 * D] = _dot(wqkv_ref[:, D:2 * D], bd).astype(BF16)
    aw[:, 2 * D:3 * D] = _dot(wqkv_ref[:, 2 * D:3 * D], perm).astype(BF16)
    awo[...] = _dot_tn(perm, awo_ref[...]).astype(BF16)

    def a_phase1(first):
        kvt[...] = jnp.zeros(kvt.shape, F32)

        def body(i, z):
            rows = pl.ds(pl.multiple_of(i * RB, RB), RB)
            if first:
                x = x_ref[rows, :].astype(F32)
                xs[rows, :] = x
            else:
                x = xs[rows, :]
            h = _ln(x).astype(BF16)
            pk = _phi(_dot(h, aw[:, D:2 * D]))
            v = _dot(h, aw[:, 2 * D:3 * D]).astype(BF16)
            pq = _phi(_dot(h, aw[:, 0:D]))
            phq[rows, :] = jnp.concatenate(pq, axis=1).astype(BF16)
            pkb = jnp.concatenate(pk, axis=1).astype(BF16)
            kvt[...] += _dot_tn(v, pkb)
            return z + jnp.sum(pkb.astype(F32), axis=0, keepdims=True)

        z = lax.fori_loop(0, S // RB, body, jnp.zeros((1, 2 * D), F32))
        rr = lax.broadcasted_iota(jnp.int32, (D, 2 * D), 0)
        cc = lax.broadcasted_iota(jnp.int32, (D, 2 * D), 1)
        kvm[...] = jnp.where((rr & 31) == (cc & 31), kvt[...], 0.0).T.astype(BF16)
        return z

    def a_phase2(z, first):
        nb = S // RB
        tpb = HD // nb

        def body(i, _):
            rows = pl.ds(pl.multiple_of(i * RB, RB), RB)
            p = phq[rows, :]
            num = _dot(p, kvm[...])
            rden = 1.0 / (_group(jnp.add, _tiles(p.astype(F32) * z)) + 1e-6)
            o = jnp.concatenate([t * rden for t in _tiles(num)], axis=1).astype(BF16)
            x = xs[rows, :] + _dot(o, awo[...])
            xs[rows, :] = x
            xn[rows, :] = _ln(x).astype(BF16).astype(F32)
            if first:
                for m in range(3):
                    src = stage[m, pl.ds(pl.multiple_of(i * tpb, tpb), tpb), :]
                    bw[m, i] = src.T
            return 0

        lax.fori_loop(0, nb, body, 0)

    def b_layer(last):
        qi = lax.broadcasted_iota(jnp.int32, (L, 128), 0)
        ln_ = lax.broadcasted_iota(jnp.int32, (L, 128), 1)
        kj = ln_ & 63
        left = ln_ < 64
        allow = (qi < M) | (qi >= kj)
        real = kj < L
        z24 = jnp.zeros((64 - L, 128), F32)
        z64 = jnp.zeros((64, 128), F32)
        ppb = NP // (S // RB)

        def big(t):
            t0, t1, t2 = _tiles(t)
            c0 = jnp.concatenate([t0, z24, z64], axis=0)
            c1 = jnp.concatenate([jnp.where(left, t1, 0.0), z24,
                                  jnp.where(left, 0.0, t1), z24], axis=0)
            c2 = jnp.concatenate([z64, t2, z24], axis=0)
            return jnp.concatenate([c0, c1, c2], axis=1).astype(BF16)

        def halves(op, fill, t):
            a = op(jnp.where(left, t, fill), axis=1, keepdims=True)
            b = op(jnp.where(left, fill, t), axis=1, keepdims=True)
            return jnp.where(left, a, b)

        def body(s, mem):
            rows = pl.ds(pl.multiple_of(s * SEG, SEG), SEG)
            h = jnp.concatenate([mem, xn[rows, :]], axis=0)

            def proj(m, j):
                o = (j % ppb) * PW
                return _dot(h, bw[m, j // ppb, :, o:o + PW])

            st = {}
            for j in range(NP + 2):
                if j < NP:
                    k = big(proj(1, j))
                    q = proj(0, j).astype(BF16).astype(F32)
                    v = big(proj(2, j))
                    st[j] = (q, k, v)
                if 1 <= j <= NP:
                    q, k, v = st[j - 1]
                    sc = _dot_nt(q, k) * (BD ** -0.5)
                    sc = jnp.where(real, jnp.where(allow, sc, -1e9), -jnp.inf)
                    e = jnp.exp(sc - halves(jnp.max, -jnp.inf, sc))
                    p = e * (1.0 / halves(jnp.sum, 0.0, e))
                    st[j - 1] = (p.astype(BF16).astype(F32), v)
                if j >= 2:
                    p, v = st.pop(j - 2)
                    osc[:, (j - 2) * PW:(j - 1) * PW] = _dot(p, v).astype(BF16).astype(F32)
            out = _dot(osc[...], bwo[...])
            x = xs[rows, :] + out[M:, :]
            if last:
                o_ref[rows, :] = x.astype(o_ref.dtype)
            else:
                xs[rows, :] = x
            return out[:M, :].astype(BF16).astype(F32)

        lax.fori_loop(0, S // SEG, body, mem0_ref[...].astype(F32))

    z = a_phase1(True)
    for c_ in cps:
        c_.wait()
    a_phase2(z, True)
    b_layer(False)
    a_phase2(a_phase1(False), False)
    b_layer(True)


@jax.jit
def pallas_interleave_layers__linear_kernel_hedgehog__memory_aug_recurrent_mem_tr__prompt_kernel(
    A_x: jax.Array,
    A_wqkv: jax.Array,
    A_w_phi: jax.Array,
    A_wo: jax.Array,
    B_x: jax.Array,
    B_mem0: jax.Array,
    B_Wq: jax.Array,
    B_Wk: jax.Array,
    B_Wv: jax.Array,
    B_Wo: jax.Array,
    B_seg_len: jax.Array,
):
    del B_x, B_seg_len
    wt = lambda w: w.transpose(1, 2, 0).reshape(HD, D)
    vm = pl.BlockSpec(memory_space=pltpu.VMEM)
    hbm = pl.BlockSpec(memory_space=pl.ANY)
    nb = S // RB
    out = pl.pallas_call(
        _kernel,
        out_shape=jax.ShapeDtypeStruct((S, D), A_x.dtype),
        in_specs=[vm] * 5 + [hbm] * 4,
        out_specs=vm,
        scratch_shapes=[
            pltpu.VMEM((S, D), F32),
            pltpu.VMEM((S, D), F32),
            pltpu.VMEM((D, 3 * D), BF16),
            pltpu.VMEM((D, D), BF16),
            pltpu.VMEM((S, 2 * D), BF16),
            pltpu.VMEM((D, 2 * D), F32),
            pltpu.VMEM((2 * D, D), BF16),
            pltpu.VMEM((128, D), BF16),
            pltpu.VMEM((3, HD, D), BF16),
            pltpu.VMEM((3, nb, D, HD // nb), BF16),
            pltpu.VMEM((HD, D), BF16),
            pltpu.VMEM((L, HD), F32),
            pltpu.SemaphoreType.DMA((4,)),
        ],
        compiler_params=pltpu.CompilerParams(vmem_limit_bytes=110 * 2**20),
        name="interleave_fused",
    )(A_x.reshape(S, D), A_wqkv, A_w_phi.transpose(1, 2, 0).reshape(AD, AH * AD), A_wo,
      B_mem0.reshape(M, D), wt(B_Wq), wt(B_Wk), wt(B_Wv), B_Wo.reshape(HD, D))
    return out.reshape(A_x.shape)
```

```python
import jax
import jax.numpy as jnp
from jax import lax
import jax.experimental.pallas as pl
import jax.experimental.pallas.tpu as pltpu

F32 = jnp.float32
BF16 = jnp.bfloat16

S, D = 2048, 640
AH, AD = 32, 20
BH, BD = 32, 192
M, SEG = 8, 32
L = M + SEG
HD = BH * BD
NP = BH // 2
PW = 2 * BD
RB = 256
NT = D // 128


def _dot(a, b):
    return lax.dot_general(a, b, (((1,), (0,)), ((), ())), preferred_element_type=F32)


def _dot_nt(a, b):
    return lax.dot_general(a, b, (((1,), (1,)), ((), ())), preferred_element_type=F32)


def _dot_tn(a, b):
    return lax.dot_general(a, b, (((0,), (0,)), ((), ())), preferred_element_type=F32)


def _ln(x):
    m = jnp.mean(x, axis=-1, keepdims=True)
    c = x - m
    v = jnp.mean(c * c, axis=-1, keepdims=True)
    return c * lax.rsqrt(v + 1e-5)


def _tiles(x):
    return [x[:, t * 128:(t + 1) * 128] for t in range(x.shape[1] // 128)]


def _group(op, tiles):
    t = tiles[0]
    for u in tiles[1:]:
        t = op(t, u)
    t = op(t, pltpu.roll(t, 64, 1))
    return op(t, pltpu.roll(t, 32, 1))


def _phi(p):
    ts = _tiles(p)
    mx = _group(jnp.maximum, ts)
    mn = _group(jnp.minimum, ts)
    ep = [jnp.exp(t - mx) for t in ts]
    en = [jnp.exp(mn - t) for t in ts]
    rp = 1.0 / _group(jnp.add, ep)
    rn = 1.0 / _group(jnp.add, en)
    return [e * rp for e in ep] + [e * rn for e in en]


def _kernel(x_ref, wqkv_ref, wp_ref, awo_ref, mem0_ref, wq_h, wk_h, wv_h, wo_h,
            o_ref,
            xs, xn, aw, awo, phq, kvt, kvm, wpp, stage, bw, bwo, osc, hb, sems):
    cps = [pltpu.make_async_copy(src, stage.at[i], sems.at[i])
           for i, src in enumerate((wq_h, wk_h, wv_h))]
    cps.append(pltpu.make_async_copy(wo_h, bwo, sems.at[3]))
    for c in cps:
        c.start()

    r = lax.broadcasted_iota(jnp.int32, (D, D), 0)
    c = lax.broadcasted_iota(jnp.int32, (D, D), 1)
    rh = (r * 3277) >> 16
    rd = r - rh * AD
    same = (c & 31) == rh
    wpp[...] = jnp.zeros(wpp.shape, BF16)
    wpp[0:AD, :] = wp_ref[...]
    r1 = lax.broadcasted_iota(jnp.int32, (D, 128), 0)
    c1 = lax.broadcasted_iota(jnp.int32, (D, 128), 1)
    sel = jnp.where(r1 - ((r1 * 3277) >> 16) * AD == c1, 1.0, 0.0).astype(BF16)
    bd = jnp.where(same, _dot(sel, wpp[...]), 0.0).astype(BF16)
    perm = jnp.where(same & ((c >> 5) == rd), 1.0, 0.0).astype(BF16)
    aw[:, 0:D] = _dot(wqkv_ref[:, 0:D], bd).astype(BF16)
    aw[:, D:2 * D] = _dot(wqkv_ref[:, D:2 * D], bd).astype(BF16)
    aw[:, 2 * D:3 * D] = _dot(wqkv_ref[:, 2 * D:3 * D], perm).astype(BF16)
    awo[...] = _dot_tn(perm, awo_ref[...]).astype(BF16)

    def a_phase1(first):
        kvt[...] = jnp.zeros(kvt.shape, F32)

        def norm(i):
            rows = pl.ds(pl.multiple_of(i * RB, RB), RB)
            if first:
                x = x_ref[rows, :].astype(F32)
                xs[rows, :] = x
            else:
                x = xs[rows, :]
            hb[...] = _ln(x).astype(BF16)

        norm(0)

        def body(i, z):
            rows = pl.ds(pl.multiple_of(i * RB, RB), RB)
            h = hb[...]
            norm(jnp.minimum(i + 1, S // RB - 1))
            pk = _phi(_dot(h, aw[:, D:2 * D]))
            v = _dot(h, aw[:, 2 * D:3 * D]).astype(BF16)
            pq = _phi(_dot(h, aw[:, 0:D]))
            phq[rows, :] = jnp.concatenate(pq, axis=1).astype(BF16)
            pkb = jnp.concatenate(pk, axis=1).astype(BF16)
            kvt[...] += _dot_tn(v, pkb)
            return z + jnp.sum(pkb.astype(F32), axis=0, keepdims=True)

        z = lax.fori_loop(0, S // RB, body, jnp.zeros((1, 2 * D), F32))
        rr = lax.broadcasted_iota(jnp.int32, (D, 2 * D), 0)
        cc = lax.broadcasted_iota(jnp.int32, (D, 2 * D), 1)
        kvm[...] = jnp.where((rr & 31) == (cc & 31), kvt[...], 0.0).T.astype(BF16)
        return z

    def a_phase2(z, first):
        nb = S // RB
        tpb = HD // nb

        def body(i, _):
            rows = pl.ds(pl.multiple_of(i * RB, RB), RB)
            p = phq[rows, :]
            num = _dot(p, kvm[...])
            rden = 1.0 / (_group(jnp.add, _tiles(p.astype(F32) * z)) + 1e-6)
            o = jnp.concatenate([t * rden for t in _tiles(num)], axis=1).astype(BF16)
            hr = RB // 2
            for u in range(2):
                rr = pl.ds(pl.multiple_of(i * RB + u * hr, hr), hr)
                x = xs[rr, :] + _dot(o[u * hr:(u + 1) * hr], awo[...])
                xs[rr, :] = x
                xn[rr, :] = _ln(x).astype(BF16).astype(F32)
            if first:
                for m in range(3):
                    src = stage[m, pl.ds(pl.multiple_of(i * tpb, tpb), tpb), :]
                    bw[m, i] = src.T
            return 0

        lax.fori_loop(0, nb, body, 0)

    def b_layer(last):
        qi = lax.broadcasted_iota(jnp.int32, (L, 128), 0)
        ln_ = lax.broadcasted_iota(jnp.int32, (L, 128), 1)
        kj = ln_ & 63
        left = ln_ < 64
        allow = (qi < M) | (qi >= kj)
        real = kj < L
        z24 = jnp.zeros((64 - L, 128), F32)
        z64 = jnp.zeros((64, 128), F32)
        cut = 12 * PW
        ppb = NP // (S // RB)

        def big(t):
            t0, t1, t2 = _tiles(t)
            c0 = jnp.concatenate([t0, z24, z64], axis=0)
            c1 = jnp.concatenate([jnp.where(left, t1, 0.0), z24,
                                  jnp.where(left, 0.0, t1), z24], axis=0)
            c2 = jnp.concatenate([z64, t2, z24], axis=0)
            return jnp.concatenate([c0, c1, c2], axis=1).astype(BF16)

        def halves(op, fill, t):
            a = op(jnp.where(left, t, fill), axis=1, keepdims=True)
            b = op(jnp.where(left, fill, t), axis=1, keepdims=True)
            return jnp.where(left, a, b)

        def body(s, mem):
            rows = pl.ds(pl.multiple_of(s * SEG, SEG), SEG)
            h = jnp.concatenate([mem, xn[rows, :]], axis=0)

            def proj(m, j):
                o = (j % ppb) * PW
                return _dot(h, bw[m, j // ppb, :, o:o + PW])

            st = {}
            for j in range(NP + 2):
                if j < NP:
                    k = big(proj(1, j))
                    q = proj(0, j).astype(BF16).astype(F32)
                    v = big(proj(2, j))
                    st[j] = (q, k, v)
                if 1 <= j <= NP:
                    q, k, v = st[j - 1]
                    sc = _dot_nt(q, k) * (BD ** -0.5)
                    sc = jnp.where(real, jnp.where(allow, sc, -1e9), -jnp.inf)
                    e = jnp.exp(sc - halves(jnp.max, -jnp.inf, sc))
                    p = e * (1.0 / halves(jnp.sum, 0.0, e))
                    st[j - 1] = (p.astype(BF16).astype(F32), v)
                if j >= NP:
                    c0, c1 = (j - NP) * cut // 2, (j - NP + 1) * cut // 2
                    part = _dot(osc[:, c0:c1], bwo[c0:c1, :])
                    out = part if j == NP else out + part
                if j >= 2:
                    p, v = st.pop(j - 2)
                    osc[:, (j - 2) * PW:(j - 1) * PW] = _dot(p, v).astype(BF16).astype(F32)
            out = out + _dot(osc[:, cut:], bwo[cut:, :])
            x = xs[rows, :] + out[M:, :]
            if last:
                o_ref[rows, :] = x.astype(o_ref.dtype)
            else:
                xs[rows, :] = x
            return out[:M, :].astype(BF16).astype(F32)

        lax.fori_loop(0, S // SEG, body, mem0_ref[...].astype(F32))

    z = a_phase1(True)
    for c_ in cps:
        c_.wait()
    a_phase2(z, True)
    b_layer(False)
    a_phase2(a_phase1(False), False)
    b_layer(True)


@jax.jit
def pallas_interleave_layers__linear_kernel_hedgehog__memory_aug_recurrent_mem_tr__prompt_kernel(
    A_x: jax.Array,
    A_wqkv: jax.Array,
    A_w_phi: jax.Array,
    A_wo: jax.Array,
    B_x: jax.Array,
    B_mem0: jax.Array,
    B_Wq: jax.Array,
    B_Wk: jax.Array,
    B_Wv: jax.Array,
    B_Wo: jax.Array,
    B_seg_len: jax.Array,
):
    del B_x, B_seg_len
    wt = lambda w: w.transpose(1, 2, 0).reshape(HD, D)
    vm = pl.BlockSpec(memory_space=pltpu.VMEM)
    hbm = pl.BlockSpec(memory_space=pl.ANY)
    nb = S // RB
    out = pl.pallas_call(
        _kernel,
        out_shape=jax.ShapeDtypeStruct((S, D), A_x.dtype),
        in_specs=[vm] * 5 + [hbm] * 4,
        out_specs=vm,
        scratch_shapes=[
            pltpu.VMEM((S, D), F32),
            pltpu.VMEM((S, D), F32),
            pltpu.VMEM((D, 3 * D), BF16),
            pltpu.VMEM((D, D), BF16),
            pltpu.VMEM((S, 2 * D), BF16),
            pltpu.VMEM((D, 2 * D), F32),
            pltpu.VMEM((2 * D, D), BF16),
            pltpu.VMEM((128, D), BF16),
            pltpu.VMEM((3, HD, D), BF16),
            pltpu.VMEM((3, nb, D, HD // nb), BF16),
            pltpu.VMEM((HD, D), BF16),
            pltpu.VMEM((L, HD), F32),
            pltpu.VMEM((RB, D), BF16),
            pltpu.SemaphoreType.DMA((4,)),
        ],
        compiler_params=pltpu.CompilerParams(vmem_limit_bytes=110 * 2**20),
        name="interleave_fused",
    )(A_x.reshape(S, D), A_wqkv, A_w_phi.transpose(1, 2, 0).reshape(AD, AH * AD), A_wo,
      B_mem0.reshape(M, D), wt(B_Wq), wt(B_Wk), wt(B_Wv), B_Wo.reshape(HD, D))
    return out.reshape(A_x.shape)
```
